```python
import jax
import jax.numpy as jnp

def _softmax(x, axis=-1):
    return jax.nn.softmax(x, axis=axis)
def _gelu(x):
    return jax.nn.gelu(x, approximate=True)
def _silu(x):
    return jax.nn.silu(x)
def _sigmoid(x):
    return jax.nn.sigmoid(x)
def _layernorm(x, axis=-1, eps=1e-5):
    m = jnp.mean(x, axis=axis, keepdims=True)
    v = jnp.var(x, axis=axis, keepdims=True)
    return (x - m) / jnp.sqrt(v + eps)
def _scatter_add(tgt, idx, src, axis=0):
    return tgt.at[idx].add(src)
def _segment_sum(src, seg, n):
    return jax.ops.segment_sum(src, seg, n)
class _Rng:
    def __init__(self, key):
        self._k = key
    def _next(self):
        self._k, sub = jax.random.split(self._k)
        return sub
    def normal(self, shape):
        return jax.random.normal(self._next(), shape, dtype=jnp.bfloat16)
    def randint(self, lo, hi, shape):
        return jax.random.randint(self._next(), shape, lo, hi, dtype=jnp.int32)
    def uniform(self, shape, lo=0.0, hi=1.0):
        return jax.random.uniform(self._next(), shape, jnp.bfloat16, lo, hi)
    def permutation(self, n):
        return jax.random.permutation(self._next(), n)


kernel_name = 'recurrent_scan__sliding_block_cached__moe_arch_mod__decode'

def setup_inputs():
    _rng = _Rng(jax.random.key(int.from_bytes(__import__("os").urandom(4), "little")))
    _w = (lambda a: (lambda t: t.astype(jnp.bfloat16) if jnp.issubdtype(t.dtype, jnp.floating) else t)(jnp.asarray(a)))
    def _A_setup():
        B, Sq, D = 1, 1, 512
        Hq, Hkv, Sk, Dh = 32, 32, 32768, 128
        assert Hq % Hkv == 0, (Hq, Hkv)
        return {
            "x": _w((lambda *s: _rng.normal(s) * 0.05)(B, Sq, D)),
            "k_cache": _w((lambda *s: _rng.normal(s) * 0.05)(B, Hkv, Sk, Dh)),
            "v_cache": _w((lambda *s: _rng.normal(s) * 0.05)(B, Hkv, Sk, Dh)),
            "wq": _w((lambda *s: _rng.normal(s) * 0.05)(D, Hq * Dh) * (D ** -0.5)),
            "wo": _w((lambda *s: _rng.normal(s) * 0.05)(Hq * Dh, D) * ((Hq * Dh) ** -0.5)),
        }
    _A_in = _A_setup()

    def _B_setup():
        B, S, D, F, C = 1, 1, 512, 1376, 1
        return {
            "x": _w((lambda *s: _rng.normal(s) * 0.05)(B, S, D)),
            "w_r": _w((lambda *s: _rng.normal(s) * 0.05)(D)),
            "w_gate": _w((lambda *s: _rng.normal(s) * 0.05)(D, F)),
            "w_up": _w((lambda *s: _rng.normal(s) * 0.05)(D, F)),
            "w_down": _w((lambda *s: _rng.normal(s) * 0.05)(F, D)),
        }
    _B_in = _B_setup()

    return {
        "A_x": _A_in["x"],
        "A_k_cache": _A_in["k_cache"],
        "A_v_cache": _A_in["v_cache"],
        "A_wq": _A_in["wq"],
        "A_wo": _A_in["wo"],
        "B_x": _B_in["x"],
        "B_w_r": _B_in["w_r"],
        "B_w_gate": _B_in["w_gate"],
        "B_w_up": _B_in["w_up"],
        "B_w_down": _B_in["w_down"],
    }

def reference(A_x, A_k_cache, A_v_cache, A_wq, A_wo, B_x, B_w_r, B_w_gate, B_w_up, B_w_down):
    def _A_ref(x, k_cache, v_cache, wq, wo):
        B, Sq, D = x.shape
        Hq, Dh = 32, 128
        Hkv, Sk = k_cache.shape[1], k_cache.shape[2]
        W = min(4096, max(256, Sk // 4))
        rep = Hq // Hkv
        q = (lambda x, *d: x.transpose(*d))((x @ wq).reshape(B, Sq, Hq, Dh), 0, 2, 1, 3)
        k = jnp.repeat(k_cache[:, :, Sk - W:, :], rep, axis=1)
        v = jnp.repeat(v_cache[:, :, Sk - W:, :], rep, axis=1)
        scores = jnp.einsum("bhqd,bhkd->bhqk", q, k) * (Dh ** -0.5)
        p = _softmax(scores, axis=-1)
        o = jnp.einsum("bhqk,bhkd->bhqd", p, v)
        return (lambda x, *d: x.transpose(*d))(o, 0, 2, 1, 3).reshape(B, Sq, Hq * Dh) @ wo

    def _B_ref(x, w_r, w_gate, w_up, w_down):
        B, S, D = x.shape
        C = 1
        r = x @ w_r
        idx = jnp.argsort(-r, axis=-1)[:, :C]
        idx_e = jnp.repeat(idx.reshape(B, C, 1), D, axis=2)
        x_sel = jnp.take_along_axis(x, idx_e, axis=1)
        g = _silu(x_sel @ w_gate)
        u = x_sel @ w_up
        y = (g * u) @ w_down
        r_sel = _sigmoid(jnp.take_along_axis(r, idx, axis=1))
        y = y * r_sel.reshape(B, C, 1)
        b_off = (jnp.arange(B) * S).reshape(B, 1)
        flat_idx = (idx + b_off).reshape(B * C)
        zero = (x * 0.0).reshape(B * S, D)
        upd = _scatter_add(zero, flat_idx, y.reshape(B * C, D), axis=0)
        return x + upd.reshape(B, S, D)

    x = A_x
    xn = _layernorm(x, axis=-1)
    s = _A_ref(xn, A_k_cache, A_v_cache, A_wq, A_wo)
    g = _silu(_B_ref(xn, B_w_r, B_w_gate, B_w_up, B_w_down))
    return x + s * g
```

```python
import functools
import jax
import jax.numpy as jnp
from jax import lax
from jax.experimental import pallas as pl
from jax.experimental.pallas import tpu as pltpu

D = 512
H = 32
DH = 128
F = 1376
SK = 32768
W = 4096
NT = (((1,), (1,)), ((), ()))


def make(NB=2, ROWS=128, out_f32=False, wunroll=1, hunroll=1, kvunroll=True):
    def kernel(x_hbm, k_hbm, v_hbm, wq_hbm, wo_hbm, wr_hbm, wg_hbm, wu_hbm, wd_hbm,
               o_ref,
               x_v, wr_v, wq_v, wo_v, wg_v, wu_v, wd_v, q_scr, kbuf, vbuf, wsem, ksem, vsem):

        def kv_start(h, slot):
            def one(c):
                r = pl.multiple_of(c * ROWS, ROWS)
                pltpu.make_async_copy(k_hbm.at[0, h, pl.ds(SK - W + r, ROWS), :], kbuf.at[slot, pl.ds(r, ROWS)], ksem.at[slot]).start(priority=0)
                pltpu.make_async_copy(v_hbm.at[0, h, pl.ds(SK - W + r, ROWS), :], vbuf.at[slot, pl.ds(r, ROWS)], vsem.at[slot]).start(priority=1)
            if kvunroll:
                for c in range(W // ROWS):
                    one(c)
            else:
                def b(c, _):
                    one(c)
                    return _
                lax.fori_loop(0, W // ROWS, b, 0)

        def k_wait(slot):
            pltpu.make_async_copy(kbuf.at[slot], kbuf.at[slot], ksem.at[slot]).wait()

        def v_wait(slot):
            pltpu.make_async_copy(vbuf.at[slot], vbuf.at[slot], vsem.at[slot]).wait()

        def rows_start(src, dst, sem, nrows, cr):
            n = nrows // cr
            assert n * cr == nrows
            half = n // 2
            def b(c, _):
                r0 = pl.multiple_of(c * cr, cr)
                r1 = pl.multiple_of((c + half) * cr, cr)
                pltpu.make_async_copy(src.at[pl.ds(r0, cr)], dst.at[pl.ds(r0, cr)], sem).start(priority=0)
                pltpu.make_async_copy(src.at[pl.ds(r1, cr)], dst.at[pl.ds(r1, cr)], sem).start(priority=1)
                return _
            lax.fori_loop(0, half, b, 0, unroll=wunroll)
            if n % 2:
                r = (n - 1) * cr
                pltpu.make_async_copy(src.at[pl.ds(r, cr)], dst.at[pl.ds(r, cr)], sem).start(priority=1)

        def wq_start():
            def b(c, _):
                r = pl.multiple_of(c * 8, 8)
                for p in (0, 1):
                    pltpu.make_async_copy(wq_hbm.at[pl.ds(r, 8), pl.ds(p * 2048, 2048)],
                                          wq_v.at[pl.ds(r, 8), pl.ds(p * 2048, 2048)], wsem.at[2]).start(priority=p)
                return _
            lax.fori_loop(0, D // 8, b, 0, unroll=wunroll)

        def full_wait(buf, sem):
            pltpu.make_async_copy(buf, buf, sem).wait()

        c_x = pltpu.make_async_copy(x_hbm, x_v, wsem.at[0])
        c_wr = pltpu.make_async_copy(wr_hbm, wr_v, wsem.at[1])
        c_x.start()
        c_wr.start(priority=1)
        wq_start()
        rows_start(wg_hbm, wg_v, wsem.at[3], F, 32)
        rows_start(wu_hbm, wu_v, wsem.at[4], F, 32)
        rows_start(wd_hbm, wd_v, wsem.at[5], F, 32)

        c_x.wait()
        x = x_v[0].astype(jnp.float32)
        mu = jnp.mean(x, axis=-1, keepdims=True)
        xc = x - mu
        var = jnp.mean(xc * xc, axis=-1, keepdims=True)
        xn = xc / jnp.sqrt(var + 1e-5)
        xn_b = xn.astype(jnp.bfloat16)
        xn8 = jnp.broadcast_to(xn_b, (8, D))

        full_wait(wq_v, wsem.at[2])
        q = jnp.dot(xn8, wq_v[...], preferred_element_type=jnp.float32)
        qb = q.astype(jnp.bfloat16)
        for h in range(H):
            q_scr[h] = qb[:, h * DH:(h + 1) * DH]

        rows_start(wo_hbm, wo_v, wsem.at[6], H * DH, 32)

        c_wr.wait()
        wr = wr_v[...].reshape(1, D).astype(jnp.float32)
        r = jnp.sum(xn_b.astype(jnp.float32) * wr, axis=-1, keepdims=True)
        full_wait(wg_v, wsem.at[3])
        g = lax.dot_general(xn8, wg_v[...], NT, preferred_element_type=jnp.float32)
        full_wait(wu_v, wsem.at[4])
        u = lax.dot_general(xn8, wu_v[...], NT, preferred_element_type=jnp.float32)
        hh = (g * jax.nn.sigmoid(g) * u).astype(jnp.bfloat16)
        full_wait(wd_v, wsem.at[5])
        y = jnp.dot(hh, wd_v[...], preferred_element_type=jnp.float32)
        y = y * jax.nn.sigmoid(r)
        xnf = xn_b.astype(jnp.float32)
        b = xnf + (xnf * 0.0 + y[0:1])
        gate = b * jax.nn.sigmoid(b)

        for i in range(NB):
            kv_start(i, i)

        full_wait(wo_v, wsem.at[6])
        scale = DH ** -0.5

        def head(h, acc):
            slot = h % NB
            k_wait(slot)
            s = lax.dot_general(q_scr[h], kbuf[slot], NT, preferred_element_type=jnp.float32) * scale
            m = jnp.max(s, axis=-1, keepdims=True)
            p = jnp.exp(s - m)
            l = jnp.sum(p, axis=-1, keepdims=True)
            v_wait(slot)
            o = jnp.dot(p.astype(jnp.bfloat16), vbuf[slot], preferred_element_type=jnp.float32)

            @pl.when(h + NB < H)
            def _():
                kv_start(h + NB, slot)
            o = (o / l).astype(jnp.bfloat16)
            woh = wo_v[pl.ds(pl.multiple_of(h * DH, DH), DH), :]
            return acc + jnp.dot(o, woh, preferred_element_type=jnp.float32)

        acc = lax.fori_loop(0, H, head, jnp.zeros((8, D), jnp.float32), unroll=hunroll)
        if out_f32:
            o_ref[0] = acc[0:1] * gate
        else:
            o_ref[0] = (x + acc[0:1] * gate).astype(o_ref.dtype)

    def fn(A_x, A_k_cache, A_v_cache, A_wq, A_wo, B_x, B_w_r, B_w_gate, B_w_up, B_w_down):
        any_spec = pl.BlockSpec(memory_space=pl.ANY)
        return pl.pallas_call(
            kernel,
            out_shape=jax.ShapeDtypeStruct((1, 1, D), jnp.float32 if out_f32 else A_x.dtype),
            in_specs=[any_spec] * 9,
            out_specs=pl.BlockSpec(memory_space=pltpu.VMEM),
            scratch_shapes=[
                pltpu.VMEM((1, 1, D), jnp.bfloat16),
                pltpu.VMEM((D,), jnp.bfloat16),
                pltpu.VMEM((D, H * DH), jnp.bfloat16),
                pltpu.VMEM((H * DH, D), jnp.bfloat16),
                pltpu.VMEM((F, D), jnp.bfloat16),
                pltpu.VMEM((F, D), jnp.bfloat16),
                pltpu.VMEM((F, D), jnp.bfloat16),
                pltpu.VMEM((H, 8, DH), jnp.bfloat16),
                pltpu.VMEM((NB, W, DH), jnp.bfloat16),
                pltpu.VMEM((NB, W, DH), jnp.bfloat16),
                pltpu.SemaphoreType.DMA((7,)),
                pltpu.SemaphoreType.DMA((NB,)),
                pltpu.SemaphoreType.DMA((NB,)),
            ],
            compiler_params=pltpu.CompilerParams(vmem_limit_bytes=100 * 1024 * 1024),
        )(A_x, A_k_cache, A_v_cache, A_wq, A_wo, B_w_r, B_w_gate.T, B_w_up.T, B_w_down)
    return fn


_impl = make(NB=3)


@jax.jit
def pallas_recurrent_scan__sliding_block_cached__moe_arch_mod__decode_kernel(
    A_x: jax.Array,
    A_k_cache: jax.Array,
    A_v_cache: jax.Array,
    A_wq: jax.Array,
    A_wo: jax.Array,
    B_x: jax.Array,
    B_w_r: jax.Array,
    B_w_gate: jax.Array,
    B_w_up: jax.Array,
    B_w_down: jax.Array,
):
    return _impl(A_x, A_k_cache, A_v_cache, A_wq, A_wo, B_x, B_w_r, B_w_gate, B_w_up, B_w_down)
```

```python
import functools
import jax
import jax.numpy as jnp
from jax import lax
from jax.experimental import pallas as pl
from jax.experimental.pallas import tpu as pltpu

D = 512
H = 32
DH = 128
F = 1376
SK = 32768
W = 4096
NT = (((1,), (1,)), ((), ()))
ROWS = 128
NCH = W // ROWS
NS = 4
QC = NCH // NS
NB = 8


def make(STEPS=((0,4),(4,8),(8,12),(12,16),(16,20),(20,24),(24,28),(28,32)), WS=(((0,1,2),),((3,4,5),),((6,),(7,))), out_f32=False, runroll=True, nocomp=False, wo_seq=True, LOOK=5, tailmode=1, noproj=False, nosemchk=False, t34=0, wsched=0, projmode=0, lastsplit=0):

    def kernel(x_hbm, k_hbm, v_hbm, wq_hbm, wo_hbm, wr_hbm, wg_hbm, wu_hbm, wd_hbm,
               o_ref,
               x_v, wr_v, wq_v, wo_v, wg_v, wu_v, wd_v, q_scr, o_scr, kbuf, vbuf, wsem, osem, ksem, vsem):

        def mult(v, m):
            return v if isinstance(v, int) else pl.multiple_of(v, m)

        def kv_chunk_start(g, c):
            slot = g & (NB - 1)
            r = mult(c * ROWS, ROWS)
            pltpu.make_async_copy(k_hbm.at[0, g, pl.ds(SK - W + r, ROWS), :], kbuf.at[slot, pl.ds(r, ROWS)], ksem.at[slot]).start(priority=0)
            pltpu.make_async_copy(v_hbm.at[0, g, pl.ds(SK - W + r, ROWS), :], vbuf.at[slot, pl.ds(r, ROWS)], vsem.at[slot]).start(priority=1)

        def rows_dma(src, dst, sem, r, cr, prio):
            r = mult(r, cr)
            pltpu.make_async_copy(src.at[pl.ds(r, cr)], dst.at[pl.ds(r, cr)], sem).start(priority=prio)

        def wo_pair(grp, i):
            rows_dma(wo_hbm, wo_v, osem.at[grp], grp * 512 + i * 32, 32, 0)
            rows_dma(wo_hbm, wo_v, osem.at[grp], grp * 512 + 256 + i * 32, 32, 1)

        def wo_head(si):
            h0, h1 = STEPS[si]
            n = (h1 - h0) * 2
            for i in range(n):
                rows_dma(wo_hbm, wo_v, osem.at[8 + si], h0 * 128 + i * 32, 32, 0)
                rows_dma(wo_hbm, wo_v, osem.at[8 + si], h0 * 128 + (n + i) * 32, 32, 1)

        def rounds(body):
            if runroll:
                for i in range(QC):
                    body(i)
            else:
                def b(i, _):
                    body(i)
                    return _
                lax.fori_loop(0, QC, b, 0)

        def period_regular(p):
            def rnd(i):
                for j in range(NS):
                    kv_chunk_start(p - j, j * QC + i)
            rounds(rnd)

        def period_tail(p):
            a = p - H
            base = (a * (a + 1)) // 2
            kv = [j for j in range(NS) if p - j < H]
            wo = [base + j for j in range(NS) if p - j >= H]
            if p < H + 2:
                for i in range(QC):
                    for j in kv[::-1]:
                        kv_chunk_start(p - j, j * QC + i)
                    for g_ in wo:
                        wo_pair(g_, i)
            else:
                for i in range(QC):
                    kv_chunk_start(p - kv[0], kv[0] * QC + i)
                    wo_pair(wo[0], i)
                for i in range(QC):
                    wo_pair(wo[1], i)
                    wo_pair(wo[2], i)
                if t34 == 0:
                  for g_ in (6, 7):
                    for i in range(QC):
                        wo_pair(g_, i)

        def wq_dma(t, prio):
            r = mult((t // 2) * 8, 8)
            c = mult((t % 2) * 2048, 2048)
            pltpu.make_async_copy(wq_hbm.at[pl.ds(r, 8), pl.ds(c, 2048)], wq_v.at[pl.ds(r, 8), pl.ds(c, 2048)], wsem.at[2]).start(priority=prio)

        def full_wait(buf, sem):
            pltpu.make_async_copy(buf, buf, sem).wait()

        c_x = pltpu.make_async_copy(x_hbm, x_v, wsem.at[0])
        c_wr = pltpu.make_async_copy(wr_hbm, wr_v, wsem.at[1])
        c_x.start()
        c_wr.start(priority=1)

        def wq_round(i, _):
            ii = 2 * i
            for s in range(4):
                r = pl.multiple_of(s * 64 + i * 8 // 2 * 1, 1) if False else None
                wq_dma2(s, i, 0)
                wq_dma2(s + 4, i, 1)
            return _

        def wq_dma2(s, i, prio):
            r = pl.multiple_of((s * 8 + lax.shift_right_logical(i, 1)) * 8, 8)
            c = pl.multiple_of((i & 1) * 2048, 2048)
            pltpu.make_async_copy(wq_hbm.at[pl.ds(r, 8), pl.ds(c, 2048)], wq_v.at[pl.ds(r, 8), pl.ds(c, 2048)], wsem.at[2]).start(priority=prio)
        lax.fori_loop(0, 16, wq_round, 0)

        def ffn_round(i, _):
            for src, dst, s in ((wg_hbm, wg_v, 3), (wu_hbm, wu_v, 4), (wd_hbm, wd_v, 5)):
                rows_dma(src, dst, wsem.at[s], i * 32, 32, 0)
                rows_dma(src, dst, wsem.at[s], (i + 21) * 32, 32, 1)
            kv_chunk_start(0, i)
            return _
        lax.fori_loop(0, 21, ffn_round, 0)
        rows_dma(wg_hbm, wg_v, wsem.at[3], 42 * 32, 32, 0)
        rows_dma(wu_hbm, wu_v, wsem.at[4], 42 * 32, 32, 1)
        rows_dma(wd_hbm, wd_v, wsem.at[5], 42 * 32, 32, 0)

        c_x.wait()
        x = x_v[0].astype(jnp.float32)
        mu = jnp.mean(x, axis=-1, keepdims=True)
        xc = x - mu
        var = jnp.mean(xc * xc, axis=-1, keepdims=True)
        xn = xc / jnp.sqrt(var + 1e-5)
        xn_b = xn.astype(jnp.bfloat16)
        xn8 = jnp.broadcast_to(xn_b, (8, D))

        full_wait(wq_v, wsem.at[2])
        q = jnp.dot(xn8, wq_v[...], preferred_element_type=jnp.float32)
        qb = q.astype(jnp.bfloat16)
        for h in range(H):
            q_scr[h] = qb[:, h * DH:(h + 1) * DH]

        for c in (21, 22, 23):
            kv_chunk_start(0, c)
        def ramp_round(i, _):
            kv_chunk_start(1, i)
            kv_chunk_start(2, i)
            kv_chunk_start(1, i + 8)
            return _
        lax.fori_loop(0, 8, ramp_round, 0)
        period_regular(3)

        c_wr.wait()
        wr = wr_v[...].reshape(1, D).astype(jnp.float32)
        r = jnp.sum(xn_b.astype(jnp.float32) * wr, axis=-1, keepdims=True)
        full_wait(wg_v, wsem.at[3])
        g = lax.dot_general(xn8, wg_v[...], NT, preferred_element_type=jnp.float32)
        full_wait(wu_v, wsem.at[4])
        u = lax.dot_general(xn8, wu_v[...], NT, preferred_element_type=jnp.float32)
        hh = (g * jax.nn.sigmoid(g) * u).astype(jnp.bfloat16)
        full_wait(wd_v, wsem.at[5])
        y = jnp.dot(hh, wd_v[...], preferred_element_type=jnp.float32)
        y = y * jax.nn.sigmoid(r)
        xnf = xn_b.astype(jnp.float32)
        b = xnf + (xnf * 0.0 + y[0:1])
        gate = b * jax.nn.sigmoid(b)

        period_regular(4)
        scale = DH ** -0.5

        def head(h, carry):
            slot = h & (NB - 1)
            full_wait(kbuf.at[slot], ksem.at[slot])
            if not nocomp:
                s = lax.dot_general(q_scr[h], kbuf[slot], NT, preferred_element_type=jnp.float32) * scale
                m = jnp.max(s, axis=-1, keepdims=True)
                p = jnp.exp(s - m)
                l = jnp.sum(p, axis=-1, keepdims=True)
            full_wait(vbuf.at[slot], vsem.at[slot])
            if not nocomp:
                o = jnp.dot(p.astype(jnp.bfloat16), vbuf[slot], preferred_element_type=jnp.float32)
                o_scr[h] = (o / l).astype(jnp.bfloat16)
            pp = h + LOOK

            @pl.when(pp < H)
            def _():
                period_regular(pp)

            def kv_loop(streams):
                def b(i, _):
                    for g_, c0 in streams:
                        kv_chunk_start(g_, c0 + i)
                    return _
                lax.fori_loop(0, QC, b, 0)

            def wo_loop(steps):
                nh = STEPS[steps[0]][1] - STEPS[steps[0]][0]
                assert all(STEPS[s_][1] - STEPS[s_][0] == nh for s_ in steps)
                n = nh * 2
                def b(i, _):
                    for s_ in steps:
                        h0 = STEPS[s_][0]
                        rows_dma(wo_hbm, wo_v, osem.at[s_], h0 * 128 + i * 32, 32, 0)
                        rows_dma(wo_hbm, wo_v, osem.at[s_], h0 * 128 + (n + i) * 32, 32, 1)
                    return _
                lax.fori_loop(0, n, b, 0)

            sched = {27: [('kv', [(31, 8), (30, 16), (29, 24)]), ('kv', [(31, 16), (30, 24)])],
                     28: [('kv', [(31, 24)])] + [('wo', t) for t in WS[0]],
                     29: [('wo', t) for t in WS[1]],
                     30: [('wo', t) for t in WS[2]]}
            for hh_, items in sched.items():
                @pl.when(h == hh_)
                def _(items=items):
                    for kind, arg in items:
                        if kind == 'kv':
                            kv_loop(arg)
                        else:
                            wo_loop(arg)
            return carry

        lax.fori_loop(0, H, head, 0)

        acc = jnp.zeros((8, D), jnp.float32)
        for si, (h0, h1) in enumerate(STEPS):
            full_wait(wo_v.at[pl.ds(h0 * 128, (h1 - h0) * 128)], osem.at[si])
            if not noproj:
                o4 = jnp.concatenate([o_scr[i] for i in range(h0, h1)], axis=1)
                acc = acc + jnp.dot(o4, wo_v[pl.ds(h0 * 128, (h1 - h0) * 128), :], preferred_element_type=jnp.float32)
        if out_f32:
            o_ref[0] = acc[0:1] * gate
        else:
            o_ref[0] = (x + acc[0:1] * gate).astype(o_ref.dtype)

    def fn(A_x, A_k_cache, A_v_cache, A_wq, A_wo, B_x, B_w_r, B_w_gate, B_w_up, B_w_down):
        any_spec = pl.BlockSpec(memory_space=pl.ANY)
        return pl.pallas_call(
            kernel,
            out_shape=jax.ShapeDtypeStruct((1, 1, D), jnp.float32 if out_f32 else A_x.dtype),
            in_specs=[any_spec] * 9,
            out_specs=pl.BlockSpec(memory_space=pltpu.VMEM),
            scratch_shapes=[
                pltpu.VMEM((1, 1, D), jnp.bfloat16),
                pltpu.VMEM((D,), jnp.bfloat16),
                pltpu.VMEM((D, H * DH), jnp.bfloat16),
                pltpu.VMEM((H * DH, D), jnp.bfloat16),
                pltpu.VMEM((F, D), jnp.bfloat16),
                pltpu.VMEM((F, D), jnp.bfloat16),
                pltpu.VMEM((F, D), jnp.bfloat16),
                pltpu.VMEM((H, 8, DH), jnp.bfloat16),
                pltpu.VMEM((H, 8, DH), jnp.bfloat16),
                pltpu.VMEM((NB, W, DH), jnp.bfloat16),
                pltpu.VMEM((NB, W, DH), jnp.bfloat16),
                pltpu.SemaphoreType.DMA((6,)),
                pltpu.SemaphoreType.DMA((12,)),
                pltpu.SemaphoreType.DMA((NB,)),
                pltpu.SemaphoreType.DMA((NB,)),
            ],
            compiler_params=pltpu.CompilerParams(vmem_limit_bytes=100 * 1024 * 1024, disable_bounds_checks=True, disable_semaphore_checks=nosemchk),
        )(A_x, A_k_cache, A_v_cache, A_wq, A_wo, B_w_r, B_w_gate.T, B_w_up.T, B_w_down)
    return fn


_impl = make(nosemchk=True, WS=(((0,1,2,3),),((4,5),(6,)),((7,),)))


@jax.jit
def pallas_recurrent_scan__sliding_block_cached__moe_arch_mod__decode_kernel(
    A_x: jax.Array,
    A_k_cache: jax.Array,
    A_v_cache: jax.Array,
    A_wq: jax.Array,
    A_wo: jax.Array,
    B_x: jax.Array,
    B_w_r: jax.Array,
    B_w_gate: jax.Array,
    B_w_up: jax.Array,
    B_w_down: jax.Array,
):
    return _impl(A_x, A_k_cache, A_v_cache, A_wq, A_wo, B_x, B_w_r, B_w_gate, B_w_up, B_w_down)
```

```python
import functools
import jax
import jax.numpy as jnp
from jax import lax
from jax.experimental import pallas as pl
from jax.experimental.pallas import tpu as pltpu

D = 512
H = 32
DH = 128
F = 1376
SK = 32768
W = 4096
NT = (((1,), (1,)), ((), ()))
G = 8
PR = W // G
NSEM = 8


def make(out_f32=False, nocomp=False, LOOK=2, RK=128, RV=64, wq1=32, wo1=32, ffn1=32,
         STEPS=((0,4),(4,8),(8,12),(12,16),(16,20),(20,24),(24,28),(28,32)),
         WS=((0,1),(2,3),(4,5),(6,7)), WSEQ=(False,False,False,True), runroll=False, tail=0, projloop=False):

    def kernel(x_hbm, k_hbm, v_hbm, wq_hbm, wo_hbm, wr_hbm, wg_hbm, wu_hbm, wd_hbm,
               o_ref,
               x_v, wr_v, wq_v, wo_v, wg_v, wu_v, wd_v, q_scr, o_scr, kbuf, vbuf, wsem, osem, ksem, vsem):

        def mult(v, m):
            return v if isinstance(v, int) else pl.multiple_of(v, m)

        def k_chunk(h, r, sem):
            r = mult(r, RK)
            pltpu.make_async_copy(k_hbm.at[0, h, pl.ds(SK - W + r, RK), :], kbuf.at[h, pl.ds(r, RK)], sem).start(priority=0)

        def v_chunk(h, r, sem):
            r = mult(r, RV)
            pltpu.make_async_copy(v_hbm.at[0, h, pl.ds(SK - W + r, RV), :], vbuf.at[h, pl.ds(r, RV)], sem).start(priority=1)

        def period_idx(p):
            if isinstance(p, int):
                return (p // G) * G, (p % G) * PR, p % NSEM
            return p & ~(G - 1), (p & (G - 1)) * PR, p & (NSEM - 1)

        def kv_period(p):
            h0, r0, si = period_idx(p)
            ratio = RK // RV
            def rnd(i):
                for s in range(G):
                    for a in range(ratio):
                        if a == ratio // 2:
                            k_chunk(h0 + s, r0 + i * RK, ksem.at[si])
                        j = s * ratio + a
                        vs = j % G
                        vr = i * ratio + j // G
                        v_chunk(h0 + vs, r0 + vr * RV, vsem.at[si])
            if runroll:
                for i in range(PR // RK):
                    rnd(i)
            else:
                def b(i, _):
                    rnd(i)
                    return _
                lax.fori_loop(0, PR // RK, b, 0)

        def kv_period_wait(p):
            h0, r0, si = period_idx(p)
            kk = kbuf.at[pl.ds(h0, G), pl.ds(mult(r0, PR), PR)]
            vv = vbuf.at[pl.ds(h0, G), pl.ds(mult(r0, PR), PR)]
            pltpu.make_async_copy(kk, kk, ksem.at[si]).wait()
            pltpu.make_async_copy(vv, vv, vsem.at[si]).wait()

        def rows_dma(src, dst, sem, r, cr, prio):
            r = mult(r, cr)
            pltpu.make_async_copy(src.at[pl.ds(r, cr)], dst.at[pl.ds(r, cr)], sem).start(priority=prio)

        def full_wait(buf, sem):
            pltpu.make_async_copy(buf, buf, sem).wait()

        c_x = pltpu.make_async_copy(x_hbm, x_v, wsem.at[0])
        c_wr = pltpu.make_async_copy(wr_hbm, wr_v, wsem.at[1])
        c_x.start()
        c_wr.start(priority=1)

        def wq_piece(s, i, prio, cols=2048):
            r = pl.multiple_of((s * 8 + lax.shift_right_logical(i, 1)) * 8, 8)
            c = pl.multiple_of((i & 1) * 2048, 2048)
            if prio == 1 and wq1 == 16:
                for hh in range(2):
                    cc = pl.multiple_of(c + hh * 1024, 1024)
                    pltpu.make_async_copy(wq_hbm.at[pl.ds(r, 8), pl.ds(cc, 1024)], wq_v.at[pl.ds(r, 8), pl.ds(cc, 1024)], wsem.at[2]).start(priority=prio)
            else:
                pltpu.make_async_copy(wq_hbm.at[pl.ds(r, 8), pl.ds(c, 2048)], wq_v.at[pl.ds(r, 8), pl.ds(c, 2048)], wsem.at[2]).start(priority=prio)

        def wq_round(i, _):
            for s in range(4):
                wq_piece(s, i, 0)
                wq_piece(s + 4, i, 1)
            return _
        lax.fori_loop(0, 16, wq_round, 0)

        kv_period(0)

        c_x.wait()
        x = x_v[0].astype(jnp.float32)
        mu = jnp.mean(x, axis=-1, keepdims=True)
        xc = x - mu
        var = jnp.mean(xc * xc, axis=-1, keepdims=True)
        xn = xc / jnp.sqrt(var + 1e-5)
        xn_b = xn.astype(jnp.bfloat16)
        xn8 = jnp.broadcast_to(xn_b, (8, D))

        full_wait(wq_v, wsem.at[2])
        q = jnp.dot(xn8, wq_v[...], preferred_element_type=jnp.float32)
        qb = q.astype(jnp.bfloat16)
        for h in range(H):
            q_scr[h] = qb[:, h * DH:(h + 1) * DH]

        for p in range(1, LOOK):
            kv_period(p)
        scale = DH ** -0.5

        def ffn_piece(src, dst, s, r, prio):
            if prio == 1 and ffn1 == 16:
                rows_dma(src, dst, wsem.at[s], r, 16, prio)
                rows_dma(src, dst, wsem.at[s], r + 16, 16, prio)
            else:
                rows_dma(src, dst, wsem.at[s], r, 32, prio)

        def ffn_issue(i0, i1, last=False):
            def b(i, _):
                for src, dst, s in ((wg_hbm, wg_v, 3), (wu_hbm, wu_v, 4), (wd_hbm, wd_v, 5)):
                    ffn_piece(src, dst, s, i * 32, 0)
                    ffn_piece(src, dst, s, (i + 21) * 32, 1)
                return _
            lax.fori_loop(i0, i1, b, 0)
            if last:
                ffn_piece(wg_hbm, wg_v, 3, 42 * 32, 0)
                ffn_piece(wu_hbm, wu_v, 4, 42 * 32, 1)
                ffn_piece(wd_hbm, wd_v, 5, 42 * 32, 0)

        def wo_pieces(grps, i0, i1):
            def b(i, _):
                for g_ in grps:
                    rows_dma(wo_hbm, wo_v, osem.at[g_], g_ * 512 + i * 32, 32, 0)
                    if wo1 == 16:
                        rows_dma(wo_hbm, wo_v, osem.at[g_], g_ * 512 + 256 + i * 32, 16, 1)
                        rows_dma(wo_hbm, wo_v, osem.at[g_], g_ * 512 + 256 + i * 32 + 16, 16, 1)
                    else:
                        rows_dma(wo_hbm, wo_v, osem.at[g_], g_ * 512 + 256 + i * 32, 32, 1)
                return _
            lax.fori_loop(i0, i1, b, 0)

        def heads(hs):
            ss = [lax.dot_general(q_scr[h], kbuf[h], NT, preferred_element_type=jnp.float32) * scale for h in hs]
            ms = [jnp.max(s, axis=-1, keepdims=True) for s in ss]
            ps = [jnp.exp(s - m) for s, m in zip(ss, ms)]
            ls = [jnp.sum(p, axis=-1, keepdims=True) for p in ps]
            os_ = [jnp.dot(p.astype(jnp.bfloat16), vbuf[h], preferred_element_type=jnp.float32) for p, h in zip(ps, hs)]
            for h, o, l in zip(hs, os_, ls):
                o_scr[h] = (o / l).astype(jnp.bfloat16)

        if tail == 0:
            SL = [lambda: ffn_issue(0, 11), lambda: ffn_issue(11, 16), lambda: ffn_issue(16, 21, True),
                  lambda: wo_pieces((0, 1, 2, 3), 0, 4), lambda: wo_pieces((0, 1, 2, 3), 4, 8)]
            post = lambda: (wo_pieces((4, 5), 0, 8), wo_pieces((6,), 0, 8), wo_pieces((7,), 0, 8))
        elif tail == 1:
            SL = [lambda: ffn_issue(0, 11), lambda: ffn_issue(11, 17), lambda: (ffn_issue(17, 21, True), wo_pieces((0, 1, 2, 3), 0, 1)),
                  lambda: wo_pieces((0, 1, 2, 3), 1, 5), lambda: (wo_pieces((0, 1, 2, 3), 5, 8), wo_pieces((4, 5), 0, 2))]
            post = lambda: (wo_pieces((4, 5), 2, 8), wo_pieces((6,), 0, 8), wo_pieces((7,), 0, 8))
        elif tail == 2:
            SL = [lambda: ffn_issue(0, 11), lambda: ffn_issue(11, 16), lambda: ffn_issue(16, 21, True),
                  lambda: wo_pieces((0, 1, 2, 3), 0, 4), lambda: (wo_pieces((0, 1, 2, 3), 4, 8), wo_pieces((4, 5), 0, 4))]
            post = lambda: (wo_pieces((4, 5), 4, 8), wo_pieces((6,), 0, 8), wo_pieces((7,), 0, 8))
        elif tail == 3:
            SL = [lambda: ffn_issue(0, 11), lambda: ffn_issue(11, 16), lambda: ffn_issue(16, 21, True),
                  lambda: wo_pieces((0, 1, 2, 3), 0, 4), lambda: (wo_pieces((0, 1, 2, 3), 4, 8), wo_pieces((4, 5), 0, 8))]
            post = lambda: (wo_pieces((6,), 0, 8), wo_pieces((7,), 0, 8))
        elif tail == 4:
            SL = [lambda: ffn_issue(0, 11), lambda: ffn_issue(11, 16), lambda: ffn_issue(16, 21, True),
                  lambda: wo_pieces((0, 1, 2, 3), 0, 4), lambda: (wo_pieces((0, 1, 2, 3), 4, 8), wo_pieces((4,), 0, 8), wo_pieces((5,), 0, 8))]
            post = lambda: (wo_pieces((6,), 0, 8), wo_pieces((7,), 0, 8))
        elif tail == 5:
            SL = [lambda: ffn_issue(0, 11), lambda: ffn_issue(11, 16), lambda: ffn_issue(16, 21, True),
                  lambda: wo_pieces((0, 1, 2, 3), 0, 4), lambda: (wo_pieces((0, 1, 2, 3), 4, 8), wo_pieces((4,), 0, 8), wo_pieces((5,), 0, 8), wo_pieces((6,), 0, 8))]
            post = lambda: (wo_pieces((7,), 0, 8))
        elif tail == 6:
            SL = [lambda: ffn_issue(0, 11), lambda: ffn_issue(11, 16), lambda: ffn_issue(16, 21, True),
                  lambda: wo_pieces((0, 1, 2, 3), 0, 5), lambda: (wo_pieces((0, 1, 2, 3), 5, 8), wo_pieces((4, 5), 0, 8), wo_pieces((6,), 0, 4))]
            post = lambda: (wo_pieces((6,), 4, 8), wo_pieces((7,), 0, 8))

        def step(u, carry):
            kv_period_wait(u)
            if not nocomp:
                @pl.when((u >= G - 1) & ((u & 1) == 1))
                def _():
                    h = u - (G - 1)
                    heads([h, h + 1])
            pp = u + LOOK

            @pl.when(pp < H)
            def _():
                kv_period(pp)

            @pl.when(u == H - 2)
            def _():
                SL[0]()
            return carry

        lax.fori_loop(0, H, step, 0)
        SL[1]()
        for i, h in enumerate((26, 28, 30)):
            if not nocomp:
                heads([h, h + 1])
            SL[2 + i]()

        c_wr.wait()
        wr = wr_v[...].reshape(1, D).astype(jnp.float32)
        r = jnp.sum(xn_b.astype(jnp.float32) * wr, axis=-1, keepdims=True)
        full_wait(wg_v, wsem.at[3])
        g = lax.dot_general(xn8, wg_v[...], NT, preferred_element_type=jnp.float32)
        full_wait(wu_v, wsem.at[4])
        u = lax.dot_general(xn8, wu_v[...], NT, preferred_element_type=jnp.float32)
        hh = (g * jax.nn.sigmoid(g) * u).astype(jnp.bfloat16)
        full_wait(wd_v, wsem.at[5])
        y = jnp.dot(hh, wd_v[...], preferred_element_type=jnp.float32)
        y = y * jax.nn.sigmoid(r)
        xnf = xn_b.astype(jnp.float32)
        b = xnf + (xnf * 0.0 + y[0:1])
        gate = b * jax.nn.sigmoid(b)

        post()
        if projloop:
            def proj(g_, acc):
                with jax.named_scope('L_proj'):
                    r0 = pl.multiple_of(g_ * 512, 512)
                    full_wait(wo_v.at[pl.ds(r0, 512)], osem.at[g_])
                    o4 = jnp.concatenate([o_scr[g_ * 4 + i] for i in range(4)], axis=1)
                    return acc + jnp.dot(o4, wo_v[pl.ds(r0, 512), :], preferred_element_type=jnp.float32)
            acc = lax.fori_loop(0, 8, proj, jnp.zeros((8, D), jnp.float32))
        else:
            acc = jnp.zeros((8, D), jnp.float32)
            for si, (h0, h1) in enumerate(STEPS):
                full_wait(wo_v.at[pl.ds(h0 * 128, (h1 - h0) * 128)], osem.at[si])
                o4 = jnp.concatenate([o_scr[i] for i in range(h0, h1)], axis=1)
                acc = acc + jnp.dot(o4, wo_v[pl.ds(h0 * 128, (h1 - h0) * 128), :], preferred_element_type=jnp.float32)
        if out_f32:
            o_ref[0] = acc[0:1] * gate
        else:
            o_ref[0] = (x + acc[0:1] * gate).astype(o_ref.dtype)

    def fn(A_x, A_k_cache, A_v_cache, A_wq, A_wo, B_x, B_w_r, B_w_gate, B_w_up, B_w_down):
        any_spec = pl.BlockSpec(memory_space=pl.ANY)
        return pl.pallas_call(
            kernel,
            out_shape=jax.ShapeDtypeStruct((1, 1, D), jnp.float32 if out_f32 else A_x.dtype),
            in_specs=[any_spec] * 9,
            out_specs=pl.BlockSpec(memory_space=pltpu.VMEM),
            scratch_shapes=[
                pltpu.VMEM((1, 1, D), jnp.bfloat16),
                pltpu.VMEM((D,), jnp.bfloat16),
                pltpu.VMEM((D, H * DH), jnp.bfloat16),
                pltpu.VMEM((H * DH, D), jnp.bfloat16),
                pltpu.VMEM((F, D), jnp.bfloat16),
                pltpu.VMEM((F, D), jnp.bfloat16),
                pltpu.VMEM((F, D), jnp.bfloat16),
                pltpu.VMEM((H, 8, DH), jnp.bfloat16),
                pltpu.VMEM((H, 8, DH), jnp.bfloat16),
                pltpu.VMEM((H, W, DH), jnp.bfloat16),
                pltpu.VMEM((H, W, DH), jnp.bfloat16),
                pltpu.SemaphoreType.DMA((6,)),
                pltpu.SemaphoreType.DMA((len(STEPS),)),
                pltpu.SemaphoreType.DMA((NSEM,)),
                pltpu.SemaphoreType.DMA((NSEM,)),
            ],
            compiler_params=pltpu.CompilerParams(vmem_limit_bytes=100 * 1024 * 1024, disable_bounds_checks=True, disable_semaphore_checks=True),
        )(A_x, A_k_cache, A_v_cache, A_wq, A_wo, B_w_r, B_w_gate.T, B_w_up.T, B_w_down)
    return fn


_impl = make(wq1=16, ffn1=16, tail=3, projloop=True)


@jax.jit
def pallas_recurrent_scan__sliding_block_cached__moe_arch_mod__decode_kernel(
    A_x: jax.Array,
    A_k_cache: jax.Array,
    A_v_cache: jax.Array,
    A_wq: jax.Array,
    A_wo: jax.Array,
    B_x: jax.Array,
    B_w_r: jax.Array,
    B_w_gate: jax.Array,
    B_w_up: jax.Array,
    B_w_down: jax.Array,
):
    return _impl(A_x, A_k_cache, A_v_cache, A_wq, A_wo, B_x, B_w_r, B_w_gate, B_w_up, B_w_down)
```

```python
import functools
import jax
import jax.numpy as jnp
from jax import lax
from jax.experimental import pallas as pl
from jax.experimental.pallas import tpu as pltpu

D = 512
H = 32
DH = 128
F = 1376
SK = 32768
W = 4096
NT = (((1,), (1,)), ((), ()))
G = 8
PR = W // G
NSEM = 8


def make(out_f32=False, nocomp=False, LOOK=2, RK=128, RV=64, wq1=32, wo1=32, ffn1=32,
         STEPS=((0,4),(4,8),(8,12),(12,16),(16,20),(20,24),(24,28),(28,32)),
         WS=((0,1),(2,3),(4,5),(6,7)), WSEQ=(False,False,False,True), runroll=False, tail=0, projloop=False, R=4, lag=30):

    def kernel(x_hbm, k_hbm, v_hbm, wq_hbm, wo_hbm, wr_hbm, wg_hbm, wu_hbm, wd_hbm,
               o_ref,
               x_v, wr_v, wq_v, wo_v, wg_v, wu_v, wd_v, q_scr, o_scr, kbuf, vbuf, wsem, osem, ksem, vsem):

        def mult(v, m):
            return v if isinstance(v, int) else pl.multiple_of(v, m)

        def k_chunk(h, r, sem):
            r = mult(r, RK)
            pltpu.make_async_copy(k_hbm.at[0, h, pl.ds(SK - W + r, RK), :], kbuf.at[h, pl.ds(r, RK)], sem).start(priority=0)

        def v_chunk(h, r, sem):
            r = mult(r, RV)
            pltpu.make_async_copy(v_hbm.at[0, h, pl.ds(SK - W + r, RV), :], vbuf.at[h, pl.ds(r, RV)], sem).start(priority=1)

        NR = PR // RK

        def round_idx(t):
            if isinstance(t, int):
                return (t // 32) * G, (t % 32) * RK, t % NSEM
            return lax.shift_right_logical(t, 5) * G, (t & 31) * RK, t & (NSEM - 1)

        def kv_round(t):
            h0, r0, si = round_idx(t)
            ratio = RK // RV
            for s in range(G):
                for a in range(ratio):
                    if a == ratio // 2:
                        k_chunk(h0 + s, r0, ksem.at[si])
                    j = s * ratio + a
                    v_chunk(h0 + j % G, r0 + (j // G) * RV, vsem.at[si])

        def kv_round_wait(t):
            h0, r0, si = round_idx(t)
            kk = kbuf.at[pl.ds(h0, G), pl.ds(mult(r0, RK), RK)]
            vv = vbuf.at[pl.ds(h0, G), pl.ds(mult(r0, RK), RK)]
            pltpu.make_async_copy(kk, kk, ksem.at[si]).wait()
            pltpu.make_async_copy(vv, vv, vsem.at[si]).wait()

        def rows_dma(src, dst, sem, r, cr, prio):
            r = mult(r, cr)
            pltpu.make_async_copy(src.at[pl.ds(r, cr)], dst.at[pl.ds(r, cr)], sem).start(priority=prio)

        def full_wait(buf, sem):
            pltpu.make_async_copy(buf, buf, sem).wait()

        c_x = pltpu.make_async_copy(x_hbm, x_v, wsem.at[0])
        c_wr = pltpu.make_async_copy(wr_hbm, wr_v, wsem.at[1])
        c_x.start()
        c_wr.start(priority=1)

        def wq_piece(s, i, prio, cols=2048):
            r = pl.multiple_of((s * 8 + lax.shift_right_logical(i, 1)) * 8, 8)
            c = pl.multiple_of((i & 1) * 2048, 2048)
            if prio == 1 and wq1 == 16:
                for hh in range(2):
                    cc = pl.multiple_of(c + hh * 1024, 1024)
                    pltpu.make_async_copy(wq_hbm.at[pl.ds(r, 8), pl.ds(cc, 1024)], wq_v.at[pl.ds(r, 8), pl.ds(cc, 1024)], wsem.at[2]).start(priority=prio)
            else:
                pltpu.make_async_copy(wq_hbm.at[pl.ds(r, 8), pl.ds(c, 2048)], wq_v.at[pl.ds(r, 8), pl.ds(c, 2048)], wsem.at[2]).start(priority=prio)

        def wq_round(i, _):
            for s in range(4):
                wq_piece(s, i, 0)
                wq_piece(s + 4, i, 1)
            return _
        lax.fori_loop(0, 16, wq_round, 0)

        for t in range(min(R, 4)):
            kv_round(t)

        c_x.wait()
        x = x_v[0].astype(jnp.float32)
        mu = jnp.mean(x, axis=-1, keepdims=True)
        xc = x - mu
        var = jnp.mean(xc * xc, axis=-1, keepdims=True)
        xn = xc / jnp.sqrt(var + 1e-5)
        xn_b = xn.astype(jnp.bfloat16)
        xn8 = jnp.broadcast_to(xn_b, (8, D))

        full_wait(wq_v, wsem.at[2])
        q = jnp.dot(xn8, wq_v[...], preferred_element_type=jnp.float32)
        qb = q.astype(jnp.bfloat16)
        for h in range(H):
            q_scr[h] = qb[:, h * DH:(h + 1) * DH]

        for t in range(4, R):
            kv_round(t)
        scale = DH ** -0.5

        def ffn_piece(src, dst, s, r, prio):
            if prio == 1 and ffn1 == 16:
                rows_dma(src, dst, wsem.at[s], r, 16, prio)
                rows_dma(src, dst, wsem.at[s], r + 16, 16, prio)
            else:
                rows_dma(src, dst, wsem.at[s], r, 32, prio)

        def ffn_issue(i0, i1, last=False):
            def b(i, _):
                for src, dst, s in ((wg_hbm, wg_v, 3), (wu_hbm, wu_v, 4), (wd_hbm, wd_v, 5)):
                    ffn_piece(src, dst, s, i * 32, 0)
                    ffn_piece(src, dst, s, (i + 21) * 32, 1)
                return _
            lax.fori_loop(i0, i1, b, 0)
            if last:
                ffn_piece(wg_hbm, wg_v, 3, 42 * 32, 0)
                ffn_piece(wu_hbm, wu_v, 4, 42 * 32, 1)
                ffn_piece(wd_hbm, wd_v, 5, 42 * 32, 0)

        def wo_pieces(grps, i0, i1):
            def b(i, _):
                for g_ in grps:
                    rows_dma(wo_hbm, wo_v, osem.at[g_], g_ * 512 + i * 32, 32, 0)
                    if wo1 == 16:
                        rows_dma(wo_hbm, wo_v, osem.at[g_], g_ * 512 + 256 + i * 32, 16, 1)
                        rows_dma(wo_hbm, wo_v, osem.at[g_], g_ * 512 + 256 + i * 32 + 16, 16, 1)
                    else:
                        rows_dma(wo_hbm, wo_v, osem.at[g_], g_ * 512 + 256 + i * 32, 32, 1)
                return _
            lax.fori_loop(i0, i1, b, 0)

        def heads(hs):
            ss = [lax.dot_general(q_scr[h], kbuf[h], NT, preferred_element_type=jnp.float32) * scale for h in hs]
            ms = [jnp.max(s, axis=-1, keepdims=True) for s in ss]
            ps = [jnp.exp(s - m) for s, m in zip(ss, ms)]
            ls = [jnp.sum(p, axis=-1, keepdims=True) for p in ps]
            os_ = [jnp.dot(p.astype(jnp.bfloat16), vbuf[h], preferred_element_type=jnp.float32) for p, h in zip(ps, hs)]
            for h, o, l in zip(hs, os_, ls):
                o_scr[h] = (o / l).astype(jnp.bfloat16)

        if tail == 0:
            SL = [lambda: ffn_issue(0, 11), lambda: ffn_issue(11, 16), lambda: ffn_issue(16, 21, True),
                  lambda: wo_pieces((0, 1, 2, 3), 0, 4), lambda: wo_pieces((0, 1, 2, 3), 4, 8)]
            post = lambda: (wo_pieces((4, 5), 0, 8), wo_pieces((6,), 0, 8), wo_pieces((7,), 0, 8))
        elif tail == 1:
            SL = [lambda: ffn_issue(0, 11), lambda: ffn_issue(11, 17), lambda: (ffn_issue(17, 21, True), wo_pieces((0, 1, 2, 3), 0, 1)),
                  lambda: wo_pieces((0, 1, 2, 3), 1, 5), lambda: (wo_pieces((0, 1, 2, 3), 5, 8), wo_pieces((4, 5), 0, 2))]
            post = lambda: (wo_pieces((4, 5), 2, 8), wo_pieces((6,), 0, 8), wo_pieces((7,), 0, 8))
        elif tail == 2:
            SL = [lambda: ffn_issue(0, 11), lambda: ffn_issue(11, 16), lambda: ffn_issue(16, 21, True),
                  lambda: wo_pieces((0, 1, 2, 3), 0, 4), lambda: (wo_pieces((0, 1, 2, 3), 4, 8), wo_pieces((4, 5), 0, 4))]
            post = lambda: (wo_pieces((4, 5), 4, 8), wo_pieces((6,), 0, 8), wo_pieces((7,), 0, 8))
        elif tail == 3:
            SL = [lambda: ffn_issue(0, 11), lambda: ffn_issue(11, 16), lambda: ffn_issue(16, 21, True),
                  lambda: wo_pieces((0, 1, 2, 3), 0, 4), lambda: (wo_pieces((0, 1, 2, 3), 4, 8), wo_pieces((4, 5), 0, 8))]
            post = lambda: (wo_pieces((6,), 0, 8), wo_pieces((7,), 0, 8))
        elif tail == 4:
            SL = [lambda: ffn_issue(0, 11), lambda: ffn_issue(11, 16), lambda: ffn_issue(16, 21, True),
                  lambda: wo_pieces((0, 1, 2, 3), 0, 4), lambda: (wo_pieces((0, 1, 2, 3), 4, 8), wo_pieces((4,), 0, 8), wo_pieces((5,), 0, 8))]
            post = lambda: (wo_pieces((6,), 0, 8), wo_pieces((7,), 0, 8))
        elif tail == 5:
            SL = [lambda: ffn_issue(0, 11), lambda: ffn_issue(11, 16), lambda: ffn_issue(16, 21, True),
                  lambda: wo_pieces((0, 1, 2, 3), 0, 4), lambda: (wo_pieces((0, 1, 2, 3), 4, 8), wo_pieces((4,), 0, 8), wo_pieces((5,), 0, 8), wo_pieces((6,), 0, 8))]
            post = lambda: (wo_pieces((7,), 0, 8))
        elif tail == 6:
            SL = [lambda: ffn_issue(0, 11), lambda: ffn_issue(11, 16), lambda: ffn_issue(16, 21, True),
                  lambda: wo_pieces((0, 1, 2, 3), 0, 5), lambda: (wo_pieces((0, 1, 2, 3), 5, 8), wo_pieces((4, 5), 0, 8), wo_pieces((6,), 0, 4))]
            post = lambda: (wo_pieces((6,), 4, 8), wo_pieces((7,), 0, 8))

        NT_ = H * NR

        def step(t, carry):
            kv_round_wait(t)
            if not nocomp:
                @pl.when((t >= 31) & ((t & 7) == 7))
                def _():
                    h = lax.shift_right_logical(t - 31, 3) * 2
                    heads([h, h + 1])
            tt = t + R

            @pl.when(tt < NT_)
            def _():
                kv_round(tt)

            @pl.when(tt == NT_)
            def _():
                SL[0]()
            return carry

        lax.fori_loop(0, NT_, step, 0)
        SL[1]()
        for i, h in enumerate((26, 28, 30)):
            if not nocomp:
                heads([h, h + 1])
            SL[2 + i]()

        c_wr.wait()
        wr = wr_v[...].reshape(1, D).astype(jnp.float32)
        r = jnp.sum(xn_b.astype(jnp.float32) * wr, axis=-1, keepdims=True)
        full_wait(wg_v, wsem.at[3])
        g = lax.dot_general(xn8, wg_v[...], NT, preferred_element_type=jnp.float32)
        full_wait(wu_v, wsem.at[4])
        u = lax.dot_general(xn8, wu_v[...], NT, preferred_element_type=jnp.float32)
        hh = (g * jax.nn.sigmoid(g) * u).astype(jnp.bfloat16)
        full_wait(wd_v, wsem.at[5])
        y = jnp.dot(hh, wd_v[...], preferred_element_type=jnp.float32)
        y = y * jax.nn.sigmoid(r)
        xnf = xn_b.astype(jnp.float32)
        b = xnf + (xnf * 0.0 + y[0:1])
        gate = b * jax.nn.sigmoid(b)

        post()
        if projloop:
            def proj(g_, acc):
                with jax.named_scope('L_proj'):
                    r0 = pl.multiple_of(g_ * 512, 512)
                    full_wait(wo_v.at[pl.ds(r0, 512)], osem.at[g_])
                    o4 = jnp.concatenate([o_scr[g_ * 4 + i] for i in range(4)], axis=1)
                    return acc + jnp.dot(o4, wo_v[pl.ds(r0, 512), :], preferred_element_type=jnp.float32)
            acc = lax.fori_loop(0, 8, proj, jnp.zeros((8, D), jnp.float32))
        else:
            acc = jnp.zeros((8, D), jnp.float32)
            for si, (h0, h1) in enumerate(STEPS):
                full_wait(wo_v.at[pl.ds(h0 * 128, (h1 - h0) * 128)], osem.at[si])
                o4 = jnp.concatenate([o_scr[i] for i in range(h0, h1)], axis=1)
                acc = acc + jnp.dot(o4, wo_v[pl.ds(h0 * 128, (h1 - h0) * 128), :], preferred_element_type=jnp.float32)
        if out_f32:
            o_ref[0] = acc[0:1] * gate
        else:
            o_ref[0] = (x + acc[0:1] * gate).astype(o_ref.dtype)

    def fn(A_x, A_k_cache, A_v_cache, A_wq, A_wo, B_x, B_w_r, B_w_gate, B_w_up, B_w_down):
        any_spec = pl.BlockSpec(memory_space=pl.ANY)
        return pl.pallas_call(
            kernel,
            out_shape=jax.ShapeDtypeStruct((1, 1, D), jnp.float32 if out_f32 else A_x.dtype),
            in_specs=[any_spec] * 9,
            out_specs=pl.BlockSpec(memory_space=pltpu.VMEM),
            scratch_shapes=[
                pltpu.VMEM((1, 1, D), jnp.bfloat16),
                pltpu.VMEM((D,), jnp.bfloat16),
                pltpu.VMEM((D, H * DH), jnp.bfloat16),
                pltpu.VMEM((H * DH, D), jnp.bfloat16),
                pltpu.VMEM((F, D), jnp.bfloat16),
                pltpu.VMEM((F, D), jnp.bfloat16),
                pltpu.VMEM((F, D), jnp.bfloat16),
                pltpu.VMEM((H, 8, DH), jnp.bfloat16),
                pltpu.VMEM((H, 8, DH), jnp.bfloat16),
                pltpu.VMEM((H, W, DH), jnp.bfloat16),
                pltpu.VMEM((H, W, DH), jnp.bfloat16),
                pltpu.SemaphoreType.DMA((6,)),
                pltpu.SemaphoreType.DMA((len(STEPS),)),
                pltpu.SemaphoreType.DMA((NSEM,)),
                pltpu.SemaphoreType.DMA((NSEM,)),
            ],
            compiler_params=pltpu.CompilerParams(vmem_limit_bytes=100 * 1024 * 1024, disable_bounds_checks=True, disable_semaphore_checks=True),
        )(A_x, A_k_cache, A_v_cache, A_wq, A_wo, B_w_r, B_w_gate.T, B_w_up.T, B_w_down)
    return fn


_impl = make(wq1=16, ffn1=16, tail=3, projloop=True, R=6)


@jax.jit
def pallas_recurrent_scan__sliding_block_cached__moe_arch_mod__decode_kernel(
    A_x: jax.Array,
    A_k_cache: jax.Array,
    A_v_cache: jax.Array,
    A_wq: jax.Array,
    A_wo: jax.Array,
    B_x: jax.Array,
    B_w_r: jax.Array,
    B_w_gate: jax.Array,
    B_w_up: jax.Array,
    B_w_down: jax.Array,
):
    return _impl(A_x, A_k_cache, A_v_cache, A_wq, A_wo, B_x, B_w_r, B_w_gate, B_w_up, B_w_down)
```

```python
import jax
import jax.numpy as jnp
from jax import lax
from jax.experimental import pallas as pl
from jax.experimental.pallas import tpu as pltpu

D = 512
H = 32
DH = 128
F = 1376
SK = 32768
W = 4096
G = 8
RK = 128
RV = 64
NROUND = (H // G) * (W // RK)
AHEAD = 6
NSEM = 8
PG = 4
NT = (((1,), (1,)), ((), ()))


def _mult(v, m):
    return v if isinstance(v, int) else pl.multiple_of(v, m)


def _kernel(x_hbm, k_hbm, v_hbm, wq_hbm, wo_hbm, wr_hbm, wg_hbm, wu_hbm, wd_hbm,
            o_ref,
            x_v, wr_v, wq_v, wo_v, wg_v, wu_v, wd_v, q_scr, o_scr, kbuf, vbuf,
            wsem, osem, ksem, vsem):
    f32, bf16 = jnp.float32, jnp.bfloat16

    def wait_all(buf, sem):
        pltpu.make_async_copy(buf, buf, sem).wait()

    def rows_dma(src, dst, sem, r, n, prio):
        r = _mult(r, n)
        pltpu.make_async_copy(src.at[pl.ds(r, n)], dst.at[pl.ds(r, n)], sem).start(priority=prio)

    def round_pos(t):
        if isinstance(t, int):
            return (t // 32) * G, (t % 32) * RK, t % NSEM
        return lax.shift_right_logical(t, 5) * G, (t & 31) * RK, t & (NSEM - 1)

    def kv_round(t):
        h0, r0, si = round_pos(t)
        for s in range(G):
            for a in range(2):
                if a == 1:
                    r = _mult(r0, RK)
                    pltpu.make_async_copy(k_hbm.at[0, h0 + s, pl.ds(SK - W + r, RK), :],
                                          kbuf.at[h0 + s, pl.ds(r, RK)], ksem.at[si]).start(priority=0)
                j = 2 * s + a
                hv, r = h0 + j % G, _mult(r0 + (j // G) * RV, RV)
                pltpu.make_async_copy(v_hbm.at[0, hv, pl.ds(SK - W + r, RV), :],
                                      vbuf.at[hv, pl.ds(r, RV)], vsem.at[si]).start(priority=1)

    def kv_round_wait(t):
        h0, r0, si = round_pos(t)
        wait_all(kbuf.at[pl.ds(h0, G), pl.ds(_mult(r0, RK), RK)], ksem.at[si])
        wait_all(vbuf.at[pl.ds(h0, G), pl.ds(_mult(r0, RK), RK)], vsem.at[si])

    def wq_round(i, carry):
        for s in range(4):
            for p in range(2):
                r = pl.multiple_of(((s + 4 * p) * 8 + lax.shift_right_logical(i, 1)) * 8, 8)
                nc = 2048 // (p + 1)
                for part in range(p + 1):
                    c = pl.multiple_of((i & 1) * 2048 + part * nc, nc)
                    pltpu.make_async_copy(wq_hbm.at[pl.ds(r, 8), pl.ds(c, nc)],
                                          wq_v.at[pl.ds(r, 8), pl.ds(c, nc)], wsem.at[2]).start(priority=p)
        return carry

    ffn = ((wg_hbm, wg_v, wsem.at[3]), (wu_hbm, wu_v, wsem.at[4]), (wd_hbm, wd_v, wsem.at[5]))

    def ffn_issue(i0, i1):
        def body(i, carry):
            for src, dst, sem in ffn:
                rows_dma(src, dst, sem, i * 32, 32, 0)
                rows_dma(src, dst, sem, (i + 21) * 32, 16, 1)
                rows_dma(src, dst, sem, (i + 21) * 32 + 16, 16, 1)
            return carry
        lax.fori_loop(i0, i1, body, 0)

    def ffn_issue_last():
        rows_dma(wg_hbm, wg_v, wsem.at[3], 42 * 32, 32, 0)
        rows_dma(wu_hbm, wu_v, wsem.at[4], 42 * 32, 16, 1)
        rows_dma(wu_hbm, wu_v, wsem.at[4], 42 * 32 + 16, 16, 1)
        rows_dma(wd_hbm, wd_v, wsem.at[5], 42 * 32, 32, 0)

    def wo_issue(groups, i0, i1):
        def body(i, carry):
            for g in groups:
                rows_dma(wo_hbm, wo_v, osem.at[g], g * PG * DH + i * 32, 32, 0)
                rows_dma(wo_hbm, wo_v, osem.at[g], g * PG * DH + 256 + i * 32, 32, 1)
            return carry
        lax.fori_loop(i0, i1, body, 0)

    c_x = pltpu.make_async_copy(x_hbm, x_v, wsem.at[0])
    c_wr = pltpu.make_async_copy(wr_hbm, wr_v, wsem.at[1])
    c_x.start()
    c_wr.start(priority=1)
    lax.fori_loop(0, 16, wq_round, 0)
    for t in range(4):
        kv_round(t)

    c_x.wait()
    x = x_v[0].astype(f32)
    xc = x - jnp.mean(x, axis=-1, keepdims=True)
    var = jnp.mean(xc * xc, axis=-1, keepdims=True)
    xn = (xc / jnp.sqrt(var + 1e-5)).astype(bf16)
    xn8 = jnp.broadcast_to(xn, (8, D))

    wait_all(wq_v, wsem.at[2])
    q = jnp.dot(xn8, wq_v[...], preferred_element_type=f32).astype(bf16)
    for h in range(H):
        q_scr[h] = q[:, h * DH:(h + 1) * DH]

    for t in range(4, AHEAD):
        kv_round(t)

    scale = DH ** -0.5

    def head_pair(h):
        hs = (h, h + 1)
        s = [lax.dot_general(q_scr[i], kbuf[i], NT, preferred_element_type=f32) * scale for i in hs]
        m = [jnp.max(a, axis=-1, keepdims=True) for a in s]
        p = [jnp.exp(a - b) for a, b in zip(s, m)]
        l = [jnp.sum(a, axis=-1, keepdims=True) for a in p]
        o = [jnp.dot(a.astype(bf16), vbuf[i], preferred_element_type=f32) for a, i in zip(p, hs)]
        for i, a, b in zip(hs, o, l):
            o_scr[i] = (a / b).astype(bf16)

    def step(t, carry):
        kv_round_wait(t)

        @pl.when((t >= 31) & ((t & 7) == 7))
        def _():
            head_pair(lax.shift_right_logical(t - 31, 3) * 2)

        @pl.when(t + AHEAD < NROUND)
        def _():
            kv_round(t + AHEAD)

        @pl.when(t + AHEAD == NROUND)
        def _():
            ffn_issue(0, 11)
        return carry

    lax.fori_loop(0, NROUND, step, 0)

    ffn_issue(11, 16)
    head_pair(26)
    ffn_issue(16, 21)
    ffn_issue_last()
    head_pair(28)
    wo_issue((0, 1, 2, 3), 0, 4)
    head_pair(30)
    wo_issue((0, 1, 2, 3), 4, 8)
    wo_issue((4, 5), 0, 8)

    c_wr.wait()
    xnf = xn.astype(f32)
    r = jnp.sum(xnf * wr_v[...].reshape(1, D).astype(f32), axis=-1, keepdims=True)
    wait_all(wg_v, wsem.at[3])
    g = lax.dot_general(xn8, wg_v[...], NT, preferred_element_type=f32)
    wait_all(wu_v, wsem.at[4])
    u = lax.dot_general(xn8, wu_v[...], NT, preferred_element_type=f32)
    hid = (g * jax.nn.sigmoid(g) * u).astype(bf16)
    wait_all(wd_v, wsem.at[5])
    y = jnp.dot(hid, wd_v[...], preferred_element_type=f32) * jax.nn.sigmoid(r)
    b = xnf + (xnf * 0.0 + y[0:1])
    gate = b * jax.nn.sigmoid(b)

    wo_issue((6,), 0, 8)
    wo_issue((7,), 0, 8)

    def proj(g, acc):
        rows = pl.ds(pl.multiple_of(g * PG * DH, PG * DH), PG * DH)
        wait_all(wo_v.at[rows], osem.at[g])
        o4 = jnp.concatenate([o_scr[g * PG + i] for i in range(PG)], axis=1)
        return acc + jnp.dot(o4, wo_v[rows, :], preferred_element_type=f32)

    acc = lax.fori_loop(0, H // PG, proj, jnp.zeros((8, D), f32))
    o_ref[0] = (x + acc[0:1] * gate).astype(o_ref.dtype)


@jax.jit
def pallas_recurrent_scan__sliding_block_cached__moe_arch_mod__decode_kernel(
    A_x: jax.Array,
    A_k_cache: jax.Array,
    A_v_cache: jax.Array,
    A_wq: jax.Array,
    A_wo: jax.Array,
    B_x: jax.Array,
    B_w_r: jax.Array,
    B_w_gate: jax.Array,
    B_w_up: jax.Array,
    B_w_down: jax.Array,
):
    del B_x
    assert A_k_cache.shape == (1, H, SK, DH) and W == min(4096, max(256, SK // 4))
    bf16 = jnp.bfloat16
    return pl.pallas_call(
        _kernel,
        out_shape=jax.ShapeDtypeStruct((1, 1, D), A_x.dtype),
        in_specs=[pl.BlockSpec(memory_space=pl.ANY)] * 9,
        out_specs=pl.BlockSpec(memory_space=pltpu.VMEM),
        scratch_shapes=[
            pltpu.VMEM((1, 1, D), bf16),
            pltpu.VMEM((D,), bf16),
            pltpu.VMEM((D, H * DH), bf16),
            pltpu.VMEM((H * DH, D), bf16),
            pltpu.VMEM((F, D), bf16),
            pltpu.VMEM((F, D), bf16),
            pltpu.VMEM((F, D), bf16),
            pltpu.VMEM((H, 8, DH), bf16),
            pltpu.VMEM((H, 8, DH), bf16),
            pltpu.VMEM((H, W, DH), bf16),
            pltpu.VMEM((H, W, DH), bf16),
            pltpu.SemaphoreType.DMA((6,)),
            pltpu.SemaphoreType.DMA((H // PG,)),
            pltpu.SemaphoreType.DMA((NSEM,)),
            pltpu.SemaphoreType.DMA((NSEM,)),
        ],
        compiler_params=pltpu.CompilerParams(
            vmem_limit_bytes=100 * 1024 * 1024,
            disable_bounds_checks=True,
            disable_semaphore_checks=True,
        ),
    )(A_x, A_k_cache, A_v_cache, A_wq, A_wo, B_w_r, B_w_gate.T, B_w_up.T, B_w_down)
```

```python
import jax
import jax.numpy as jnp
from jax import lax
from jax.experimental import pallas as pl
from jax.experimental.pallas import tpu as pltpu

D = 512
H = 32
DH = 128
F = 1376
SK = 32768
W = 4096
G = 8
RK = 128
RV = 64
NROUND = (H // G) * (W // RK)
AHEAD = 6
NSEM = 8
PG = 4
NT = (((1,), (1,)), ((), ()))


def _mult(v, m):
    return v if isinstance(v, int) else pl.multiple_of(v, m)


def _kernel(x_hbm, k_hbm, v_hbm, wq_hbm, wo_hbm, wr_hbm, wg_hbm, wu_hbm, wd_hbm,
            o_ref,
            x_v, wr_v, wq_v, wo_v, wg_v, wu_v, wd_v, q_scr, o_scr, kbuf, vbuf,
            wsem, osem, ksem, vsem):
    f32, bf16 = jnp.float32, jnp.bfloat16

    def wait_all(buf, sem):
        pltpu.make_async_copy(buf, buf, sem).wait()

    def rows_dma(src, dst, sem, r, n, prio):
        r = _mult(r, n)
        pltpu.make_async_copy(src.at[pl.ds(r, n)], dst.at[pl.ds(r, n)], sem).start(priority=prio)

    def round_pos(t):
        if isinstance(t, int):
            return (t // 32) * G, (t % 32) * RK, t % NSEM
        return lax.shift_right_logical(t, 5) * G, (t & 31) * RK, t & (NSEM - 1)

    def kv_copies(t):
        h0, r0, si = round_pos(t)
        out = []
        for s in range(G):
            for a in range(2):
                if a == 1:
                    r = _mult(r0, RK)
                    out.append((pltpu.make_async_copy(
                        k_hbm.at[0, h0 + s, pl.ds(SK - W + r, RK), :],
                        kbuf.at[h0 + s, pl.ds(r, RK)], ksem.at[si]), 0))
                j = 2 * s + a
                hv, r = h0 + j % G, _mult(r0 + (j // G) * RV, RV)
                out.append((pltpu.make_async_copy(
                    v_hbm.at[0, hv, pl.ds(SK - W + r, RV), :],
                    vbuf.at[hv, pl.ds(r, RV)], vsem.at[si]), 1))
        return out

    def kv_round(t):
        for c, prio in kv_copies(t):
            c.start(priority=prio)

    def kv_round_wait(t):
        for c, _ in kv_copies(t):
            c.wait()

    def wq_round(i, carry):
        for s in range(4):
            for p in range(2):
                r = pl.multiple_of(((s + 4 * p) * 8 + lax.shift_right_logical(i, 1)) * 8, 8)
                nc = 2048 // (p + 1)
                for part in range(p + 1):
                    c = pl.multiple_of((i & 1) * 2048 + part * nc, nc)
                    pltpu.make_async_copy(wq_hbm.at[pl.ds(r, 8), pl.ds(c, nc)],
                                          wq_v.at[pl.ds(r, 8), pl.ds(c, nc)], wsem.at[2]).start(priority=p)
        return carry

    ffn = ((wg_hbm, wg_v, wsem.at[3]), (wu_hbm, wu_v, wsem.at[4]), (wd_hbm, wd_v, wsem.at[5]))

    def ffn_issue(i0, i1):
        def body(i, carry):
            for src, dst, sem in ffn:
                rows_dma(src, dst, sem, i * 32, 32, 0)
                rows_dma(src, dst, sem, (i + 21) * 32, 16, 1)
                rows_dma(src, dst, sem, (i + 21) * 32 + 16, 16, 1)
            return carry
        lax.fori_loop(i0, i1, body, 0)

    def ffn_issue_last():
        rows_dma(wg_hbm, wg_v, wsem.at[3], 42 * 32, 32, 0)
        rows_dma(wu_hbm, wu_v, wsem.at[4], 42 * 32, 16, 1)
        rows_dma(wu_hbm, wu_v, wsem.at[4], 42 * 32 + 16, 16, 1)
        rows_dma(wd_hbm, wd_v, wsem.at[5], 42 * 32, 32, 0)

    def wo_issue(groups, i0, i1):
        def body(i, carry):
            for g in groups:
                rows_dma(wo_hbm, wo_v, osem.at[g], g * PG * DH + i * 32, 32, 0)
                rows_dma(wo_hbm, wo_v, osem.at[g], g * PG * DH + 256 + i * 32, 32, 1)
            return carry
        lax.fori_loop(i0, i1, body, 0)

    c_x = pltpu.make_async_copy(x_hbm, x_v, wsem.at[0])
    c_wr = pltpu.make_async_copy(wr_hbm, wr_v, wsem.at[1])
    c_x.start()
    c_wr.start(priority=1)
    lax.fori_loop(0, 16, wq_round, 0)
    for t in range(4):
        kv_round(t)

    c_x.wait()
    x = x_v[0].astype(f32)
    xc = x - jnp.mean(x, axis=-1, keepdims=True)
    var = jnp.mean(xc * xc, axis=-1, keepdims=True)
    xn = (xc / jnp.sqrt(var + 1e-5)).astype(bf16)
    xn8 = jnp.broadcast_to(xn, (8, D))

    wait_all(wq_v, wsem.at[2])
    q = jnp.dot(xn8, wq_v[...], preferred_element_type=f32).astype(bf16)
    for h in range(H):
        q_scr[h] = q[:, h * DH:(h + 1) * DH]

    for t in range(4, AHEAD):
        kv_round(t)

    scale = DH ** -0.5

    def head_pair(h):
        hs = (h, h + 1)
        s = [lax.dot_general(q_scr[i], kbuf[i], NT, preferred_element_type=f32) * scale for i in hs]
        m = [jnp.max(a, axis=-1, keepdims=True) for a in s]
        p = [jnp.exp(a - b) for a, b in zip(s, m)]
        l = [jnp.sum(a, axis=-1, keepdims=True) for a in p]
        o = [jnp.dot(a.astype(bf16), vbuf[i], preferred_element_type=f32) for a, i in zip(p, hs)]
        for i, a, b in zip(hs, o, l):
            o_scr[i] = (a / b).astype(bf16)

    def step(t, carry):
        kv_round_wait(t)

        @pl.when((t >= 31) & ((t & 7) == 7))
        def _():
            head_pair(lax.shift_right_logical(t - 31, 3) * 2)

        @pl.when(t + AHEAD < NROUND)
        def _():
            kv_round(t + AHEAD)

        @pl.when(t + AHEAD == NROUND)
        def _():
            ffn_issue(0, 11)
        return carry

    lax.fori_loop(0, NROUND, step, 0)

    ffn_issue(11, 16)
    head_pair(26)
    ffn_issue(16, 21)
    ffn_issue_last()
    head_pair(28)
    wo_issue((0, 1, 2, 3), 0, 4)
    head_pair(30)
    wo_issue((0, 1, 2, 3), 4, 8)
    wo_issue((4, 5), 0, 8)

    c_wr.wait()
    xnf = xn.astype(f32)
    r = jnp.sum(xnf * wr_v[...].reshape(1, D).astype(f32), axis=-1, keepdims=True)
    wait_all(wg_v, wsem.at[3])
    g = lax.dot_general(xn8, wg_v[...], NT, preferred_element_type=f32)
    wait_all(wu_v, wsem.at[4])
    u = lax.dot_general(xn8, wu_v[...], NT, preferred_element_type=f32)
    hid = (g * jax.nn.sigmoid(g) * u).astype(bf16)
    wait_all(wd_v, wsem.at[5])
    y = jnp.dot(hid, wd_v[...], preferred_element_type=f32) * jax.nn.sigmoid(r)
    b = xnf + (xnf * 0.0 + y[0:1])
    gate = b * jax.nn.sigmoid(b)

    wo_issue((6,), 0, 8)
    wo_issue((7,), 0, 8)

    def proj(g, acc):
        rows = pl.ds(pl.multiple_of(g * PG * DH, PG * DH), PG * DH)
        wait_all(wo_v.at[rows], osem.at[g])
        o4 = jnp.concatenate([o_scr[g * PG + i] for i in range(PG)], axis=1)
        return acc + jnp.dot(o4, wo_v[rows, :], preferred_element_type=f32)

    acc = lax.fori_loop(0, H // PG, proj, jnp.zeros((8, D), f32))
    o_ref[0] = (x + acc[0:1] * gate).astype(o_ref.dtype)


@jax.jit
def pallas_recurrent_scan__sliding_block_cached__moe_arch_mod__decode_kernel(
    A_x: jax.Array,
    A_k_cache: jax.Array,
    A_v_cache: jax.Array,
    A_wq: jax.Array,
    A_wo: jax.Array,
    B_x: jax.Array,
    B_w_r: jax.Array,
    B_w_gate: jax.Array,
    B_w_up: jax.Array,
    B_w_down: jax.Array,
):
    del B_x
    assert A_k_cache.shape == (1, H, SK, DH) and W == min(4096, max(256, SK // 4))
    bf16 = jnp.bfloat16
    return pl.pallas_call(
        _kernel,
        out_shape=jax.ShapeDtypeStruct((1, 1, D), A_x.dtype),
        in_specs=[pl.BlockSpec(memory_space=pl.ANY)] * 9,
        out_specs=pl.BlockSpec(memory_space=pltpu.VMEM),
        scratch_shapes=[
            pltpu.VMEM((1, 1, D), bf16),
            pltpu.VMEM((D,), bf16),
            pltpu.VMEM((D, H * DH), bf16),
            pltpu.VMEM((H * DH, D), bf16),
            pltpu.VMEM((F, D), bf16),
            pltpu.VMEM((F, D), bf16),
            pltpu.VMEM((F, D), bf16),
            pltpu.VMEM((H, 8, DH), bf16),
            pltpu.VMEM((H, 8, DH), bf16),
            pltpu.VMEM((H, W, DH), bf16),
            pltpu.VMEM((H, W, DH), bf16),
            pltpu.SemaphoreType.DMA((6,)),
            pltpu.SemaphoreType.DMA((H // PG,)),
            pltpu.SemaphoreType.DMA((NSEM,)),
            pltpu.SemaphoreType.DMA((NSEM,)),
        ],
        compiler_params=pltpu.CompilerParams(
            vmem_limit_bytes=100 * 1024 * 1024,
        ),
    )(A_x, A_k_cache, A_v_cache, A_wq, A_wo, B_w_r, B_w_gate.T, B_w_up.T, B_w_down)
```
